```python
import os as _os
_os.environ.setdefault("JAX_PLATFORMS", "cpu")
import jax
import jax.numpy as jnp

def _softmax(x, axis=-1):
    return jax.nn.softmax(x, axis=axis)
def _gelu(x):
    return jax.nn.gelu(x, approximate=True)
def _silu(x):
    return jax.nn.silu(x)
def _sigmoid(x):
    return jax.nn.sigmoid(x)
def _layernorm(x, axis=-1, eps=1e-5):
    m = jnp.mean(x, axis=axis, keepdims=True)
    v = jnp.var(x, axis=axis, keepdims=True)
    return (x - m) / jnp.sqrt(v + eps)
def _scatter_add(tgt, idx, src, axis=0):
    return tgt.at[idx].add(src)
def _segment_sum(src, seg, n):
    return jax.ops.segment_sum(src, seg, n)
class _Rng:
    def __init__(self, key):
        self._k = key
    def _next(self):
        self._k, sub = jax.random.split(self._k)
        return sub
    def normal(self, shape):
        return jax.random.normal(self._next(), shape, dtype=jnp.bfloat16)
    def randint(self, lo, hi, shape):
        return jax.random.randint(self._next(), shape, lo, hi, dtype=jnp.int32)
    def uniform(self, shape, lo=0.0, hi=1.0):
        return jax.random.uniform(self._next(), shape, jnp.bfloat16, lo, hi)
    def permutation(self, n):
        return jax.random.permutation(self._next(), n)


kernel_name = 'concat_heads__spectral_gfnet__mha_block__prompt'

def setup_inputs():
    _rng = _Rng(jax.random.key(int.from_bytes(__import__("os").urandom(4), "little")))
    _w = (lambda a: (lambda t: t.astype(jnp.bfloat16) if jnp.issubdtype(t.dtype, jnp.floating) else t)(jnp.asarray(a)))
    def _A_setup():
        B, S, D = 1, 2048, 576
        Df = D // 2 + 1
        return {
            "x": _w((lambda *s: _rng.normal(s) * 0.05)(B, S, D)),
            "w_r": _w((lambda *s: _rng.normal(s) * 0.05)(S, Df) * 0.02),
            "w_i": _w((lambda *s: _rng.normal(s) * 0.05)(S, Df) * 0.02),
        }
    _A_in = _A_setup()

    def _B_setup():
        B, S, D, H = 1, 2048, 576, 32
        return {
            "x": _w((lambda *s: _rng.normal(s) * 0.1)(B, S, D)),
            "wqkv": _w((lambda *s: _rng.normal(s) * 0.1)(D, 3 * D)),
            "wo": _w((lambda *s: _rng.normal(s) * 0.05)(D, D)),
        }
    _B_in = _B_setup()

    return {
        "A_x": _A_in["x"],
        "A_w_r": _A_in["w_r"],
        "A_w_i": _A_in["w_i"],
        "B_x": _B_in["x"],
        "B_wqkv": _B_in["wqkv"],
        "B_wo": _B_in["wo"],
    }

def reference(A_x, A_w_r, A_w_i, B_x, B_wqkv, B_wo):
    def _A_ref(x, w_r, w_i):
        B, S, D = x.shape
        X = (lambda x, axes=(-2,-1): jnp.fft.rfft2(x.astype(jnp.float32), axes=axes))(x, axes=(-2, -1))
        W = w_r + 1j * w_i
        X = X * W
        y = (lambda x, s, axes=(-2,-1): jnp.fft.irfft2(x, s=s, axes=axes).astype(jnp.bfloat16))(X, (S, D), axes=(-2, -1))
        return y

    def _B_ref(x, wqkv, wo):
        B, S, D = x.shape
        H = 32
        Dh = D // H
        qkv = (lambda x, *d: x.transpose(*d))((x @ wqkv).reshape(B, S, 3, H, Dh), 2, 0, 3, 1, 4)
        q, k, v = qkv[0], qkv[1], qkv[2]
        scores = jnp.einsum("bhqd,bhkd->bhqk", q, k) * (Dh ** -0.5)
        p = _softmax(scores, axis=-1)
        o = jnp.einsum("bhqk,bhkd->bhqd", p, v)
        return (lambda x, *d: x.transpose(*d))(o, 0, 2, 1, 3).reshape(B, S, D) @ wo

    a = _A_ref(A_x, A_w_r, A_w_i)
    b = _B_ref(B_x, B_wqkv, B_wo)
    return jnp.concatenate([a, b], axis=-1)
```

```python
import numpy as np
import jax
import jax.numpy as jnp
from jax import lax
import jax.experimental.pallas as pl
import jax.experimental.pallas.tpu as pltpu

S, D, H = 2048, 576, 32
DH = D // H
DF = D // 2 + 1
RP = 296
RZ = 360
NT = S // 128
N1, N2 = 9, 64
F32, BF16 = jnp.float32, jnp.bfloat16
QB = 512
KC = 128
HG = 8
VR = 24
NC = S // QB
BIAS = 0.7
NG = H // HG
OB = 256


def _constants():
    d2 = np.arange(N2)[None, :]
    fwd = np.zeros((5, 128, 128))
    inv = np.zeros((5, 128, 128))
    norm = 1.0 / (S * D)
    kd = (N1 * np.arange(33))[:, None]
    ang = 2.0 * np.pi * ((kd * d2) % D) / D
    fwd[0, 0:33, 0:64] = np.cos(ang)
    fwd[0, 40:73, 0:64] = -np.sin(ang)
    c = np.full((33, 1), 2.0)
    c[0] = c[32] = 1.0
    inv[0, 0:64, 0:33] = (c * np.cos(ang)).T * norm
    inv[0, 0:64, 40:73] = (-c * np.sin(ang)).T * norm
    inv[0, 0:64, 40] = 0.0
    inv[0, 0:64, 72] = 0.0
    for r in range(1, 5):
        for j, (cls, sg) in enumerate(((r, 1.0), (N1 - r, -1.0))):
            kd = (cls + N1 * np.arange(32))[:, None]
            ang = 2.0 * np.pi * ((kd * d2) % D) / D
            co, si = np.cos(ang), -np.sin(ang)
            fwd[r, 32 * j:32 * j + 32, 0:64] = co
            fwd[r, 32 * j:32 * j + 32, 64:128] = -sg * si
            fwd[r, 64 + 32 * j:64 + 32 * j + 32, 0:64] = si
            fwd[r, 64 + 32 * j:64 + 32 * j + 32, 64:128] = sg * co
            inv[r, 0:64, 32 * j:32 * j + 32] = 2 * norm * co.T
            inv[r, 0:64, 64 + 32 * j:64 + 32 * j + 32] = 2 * norm * si.T
            inv[r, 64:128, 32 * j:32 * j + 32] = -sg * 2 * norm * si.T
            inv[r, 64:128, 64 + 32 * j:64 + 32 * j + 32] = sg * 2 * norm * co.T
    k1 = np.arange(NT)[:, None, None]
    s2 = np.arange(128)[None, :, None]
    k2 = np.arange(128)[None, None, :]
    a = 2.0 * np.pi * (((k1 + NT * k2) * s2) % S) / S
    g = np.stack([np.cos(a), -np.sin(a)], axis=1)
    return np.concatenate([fwd, inv], axis=0).astype(np.float32), g.astype(np.float32)


def _fft16(re, im, sign):
    n = len(re)
    if n == 1:
        return re, im
    er, ei = _fft16(re[0::2], im[0::2], sign)
    orr, oi = _fft16(re[1::2], im[1::2], sign)
    outr, outi = [None] * n, [None] * n
    for k in range(n // 2):
        if k == 0:
            pr, pi_ = er[k] + orr[k], ei[k] + oi[k]
            mr, mi = er[k] - orr[k], ei[k] - oi[k]
        elif 4 * k == n:
            if sign > 0:
                pr, pi_ = er[k] - oi[k], ei[k] + orr[k]
                mr, mi = er[k] + oi[k], ei[k] - orr[k]
            else:
                pr, pi_ = er[k] + oi[k], ei[k] - orr[k]
                mr, mi = er[k] - oi[k], ei[k] + orr[k]
        else:
            wr = float(np.cos(2 * np.pi * k / n))
            wi = float(sign * np.sin(2 * np.pi * k / n))
            if 8 * k == n or 8 * k == 3 * n:
                same = (wi > 0) == (wr > 0)
                if same:
                    tr, ti = (orr[k] - oi[k]) * wr, (orr[k] + oi[k]) * wr
                else:
                    tr, ti = (orr[k] + oi[k]) * wr, (oi[k] - orr[k]) * wr
            else:
                tr = orr[k] * wr - oi[k] * wi
                ti = orr[k] * wi + oi[k] * wr
            pr, pi_ = er[k] + tr, ei[k] + ti
            mr, mi = er[k] - tr, ei[k] - ti
        outr[k], outi[k] = pr, pi_
        outr[k + n // 2], outi[k + n // 2] = mr, mi
    return outr, outi


_C9 = [float(np.cos(2 * np.pi * b / N1)) for b in range(5)]
_S9 = [float(np.sin(2 * np.pi * b / N1)) for b in range(5)]


def _mm(a, b):
    return lax.dot_general(a, b, (((1,), (0,)), ((), ())), preferred_element_type=F32)


def _mm_nt(a, b):
    return lax.dot_general(a, b, (((1,), (1,)), ((), ())), preferred_element_type=F32)


def _interleave(*streams):
    keyed = []
    for si, st in enumerate(streams):
        for i, f in enumerate(st):
            keyed.append(((i + 0.5) / len(st) * (1.0 if si == 0 else BIAS), si, i, f))
    for _, _, _, f in sorted(keyed, key=lambda e: e[:3]):
        f()


def _kernel(xa_hbm, wr_hbm, wi_hbm, xb_hbm, wqkv_hbm, wo_hbm, dm_hbm, g_hbm,
            out_hbm,
            xa_v, wr_v, wi_v, xb_v, wqkv_v, wo_v, dm_v, g_v,
            wt_v, wot_v, qt_v, kt_v, kw_v, vt_v, ot_v, a9_v, b9_v, z_v, wp_v, tail_v, outa_v, outb_v,
            sems, osems):
    def ds(i, n):
        return pl.ds(i * n, n) if isinstance(i, int) else pl.ds(pl.multiple_of(i * n, n), n)

    def cp_xb(c):
        return pltpu.make_async_copy(xb_hbm.at[:, ds(c, QB)], xb_v.at[:, ds(c, QB)], sems.at[1 + c])

    def cp_xa(c):
        return pltpu.make_async_copy(xa_hbm.at[:, ds(c, QB)], xa_v.at[:, ds(c, QB)], sems.at[5 + c])

    cp_w = pltpu.make_async_copy(wqkv_hbm.at[:, pl.ds(0, 2 * D)], wqkv_v.at[:, pl.ds(0, 2 * D)], sems.at[0])
    cp_wv = pltpu.make_async_copy(wqkv_hbm.at[:, pl.ds(2 * D, D)], wqkv_v.at[:, pl.ds(2 * D, D)], sems.at[14])
    cp_dm = pltpu.make_async_copy(dm_hbm, dm_v, sems.at[9])
    cp_g = pltpu.make_async_copy(g_hbm, g_v, sems.at[10])
    cp_wr = pltpu.make_async_copy(wr_hbm, wr_v, sems.at[11])
    cp_wi = pltpu.make_async_copy(wi_hbm, wi_v, sems.at[12])
    cp_wo = pltpu.make_async_copy(wo_hbm, wo_v, sems.at[13])

    qscale = float(DH ** -0.5 * np.log2(np.e))
    MB = 192

    def qk_units(c):
        def unit(mb):
            def run():
                t = _mm(wt_v[mb * MB:(mb + 1) * MB, :], xb_v[:, ds(c, QB)])
                sec, r0 = divmod(mb * MB, D)
                if sec == 1:
                    qt_v[r0:r0 + MB, ds(c, QB)] = (t * qscale).astype(BF16)
                    i = r0 // MB
                    for w in range(3 * i, 3 * i + 3):
                        kw_v[w, ds(c, QB), :] = kt_v[64 * w:64 * w + 128, ds(c, QB)].T
                else:
                    kt_v[r0:r0 + MB, ds(c, QB)] = t.astype(BF16)
            return run
        return [unit(mb) for mb in range(6)]

    def v_units(c):
        def unit(mb):
            def run():
                vt_v[mb * MB:(mb + 1) * MB, ds(c, QB)] = _mm(wt_v[2 * D + mb * MB:2 * D + (mb + 1) * MB, :],
                                                             xb_v[:, ds(c, QB)])
            return run
        return [unit(mb) for mb in range(3)]

    def fwd9_units(c):
        def unit(i, rb):
            def run():
                ls = pl.ds(pl.multiple_of(c * QB + i * 128, 128), 128)
                rs = slice(16 * rb, 16 * rb + 16)
                x = [xa_v[N2 * d1 + 16 * rb:N2 * d1 + 16 * rb + 16, ls].astype(F32) for d1 in range(N1)]
                sm = [None] + [x[j] + x[N1 - j] for j in range(1, 5)]
                df = [None] + [x[j] - x[N1 - j] for j in range(1, 5)]
                a9_v[0, rs, ls] = (x[0] + sm[1] + sm[2] + sm[3] + sm[4]).astype(BF16)
                for r in range(1, 5):
                    re, im = x[0], None
                    for j in range(1, 5):
                        jr = (j * r) % N1
                        co = _C9[min(jr, N1 - jr)]
                        si = -_S9[jr] if jr < 5 else _S9[N1 - jr]
                        re = re + sm[j] * co
                        im = df[j] * si if im is None else im + df[j] * si
                    a9_v[r, rs, ls] = re.astype(BF16)
                    a9_v[r, 64 + 16 * rb:64 + 16 * rb + 16, ls] = im.astype(BF16)
            return run
        return [unit(i, rb) for i in range(QB // 128) for rb in range(4)]

    def fwd64(c, carry):
        for r in range(5):
            if r == 0:
                z = _mm(dm_v[0, 0:80, 0:64], a9_v[0, 0:64, ds(c, QB)])
                parts = ((0, 0, 40), (RZ, 40, 40))
            else:
                z = _mm(dm_v[r], a9_v[r, :, ds(c, QB)])
                parts = ((r, 0, 32), (N1 - r, 32, 32), (RZ + r, 64, 32), (RZ + N1 - r, 96, 32))
            for i in range(QB // 128):
                for dst, src, n in parts:
                    z_v[c * 4 + i, pl.ds(dst, n, stride=N1), :] = z[src:src + n, i * 128:(i + 1) * 128]
        return carry

    def fft16(rg, sign):
        r0 = rg * 8 if isinstance(rg, int) else pl.multiple_of(rg * 8, 8)
        re = [z_v[t, pl.ds(r0, 8), :] for t in range(NT)]
        im = [z_v[t, pl.ds(RZ + r0, 8), :] for t in range(NT)]
        re, im = _fft16(re, im, sign)
        for t in range(NT):
            z_v[t, pl.ds(r0, 8), :] = re[t]
            z_v[t, pl.ds(RZ + r0, 8), :] = im[t]

    def fft16_v(half, sign):
        def step(i, carry):
            _interleave(v_units(2 * half + i),
                        [(lambda j=j: fft16(i * 18 + j, sign)) for j in range(18)],
                        *([wperm1_units(2 * i) + wperm1_units(2 * i + 1)] if half == 0 else []))
            return carry
        lax.fori_loop(0, 2, step, 0)
        fft16(36, sign)

    def wperm1_units(c):
        def unit(i, t):
            def run():
                src = (wr_v, wi_v)[i]
                ls = pl.ds(pl.multiple_of(c * QB + t * 128, 128), 128)
                lo = pltpu.bitcast(src[0:256, ls], jnp.uint32)
                hi = jnp.concatenate([src[256:DF, ls], jnp.zeros((320 - DF, 128), BF16)], axis=0)
                hi = pltpu.bitcast(hi, jnp.uint32)
                wp_v[2 * i, ls, :] = lo.T
                wp_v[2 * i + 1, ls, :] = jnp.concatenate([hi, jnp.zeros((96, 128), jnp.uint32)], axis=0).T
            return run
        return [unit(i, t) for i in range(2) for t in range(QB // 128)]

    def filt(k1, i):
        lo = wp_v[2 * i, pl.ds(k1, 128, stride=NT), :].T
        hi = wp_v[2 * i + 1, pl.ds(k1, 128, stride=NT), :].T[0:32]
        return jnp.concatenate([pltpu.bitcast(lo, BF16).astype(F32),
                                pltpu.bitcast(hi, BF16).astype(F32)[0:RP - 256]], axis=0)

    GU = 4

    def gstep(i, carry):
        ys = []
        for u in range(GU):
            k1 = i * GU + u
            a = jnp.concatenate([z_v[k1, 0:RP, :], z_v[k1, RZ:RZ + RP, :]], axis=0)
            pr = _mm(a, g_v[k1, 0])
            pi_ = _mm(a, g_v[k1, 1])
            xr = pr[:RP] - pi_[RP:]
            xi = pi_[:RP] + pr[RP:]
            wr, wi = filt(k1, 0), filt(k1, 1)
            ys.append(jnp.concatenate([xr * wr - xi * wi, xr * wi + xi * wr], axis=0))
        for u in range(GU):
            k1 = i * GU + u
            qr = _mm_nt(ys[u], g_v[k1, 0])
            qi = _mm_nt(ys[u], g_v[k1, 1])
            z_v[k1, 0:RP, :] = qr[:RP] + qi[RP:]
            z_v[k1, RZ:RZ + RP, :] = qr[RP:] - qi[:RP]
        return carry

    def inv64(c, carry):
        for r in range(5):
            if r == 0:
                parts = ((0, 40), (RZ, 40))
            else:
                parts = ((r, 32), (N1 - r, 32), (RZ + r, 32), (RZ + N1 - r, 32))
            y = jnp.concatenate(
                [jnp.concatenate([z_v[c * 4 + i, pl.ds(st, n, stride=N1), :] for st, n in parts], axis=0)
                 for i in range(QB // 128)], axis=1).astype(BF16)
            if r == 0:
                b9_v[0, 0:64, ds(c, QB)] = _mm(dm_v[5, 0:64, 0:80], y)
            else:
                b9_v[r, :, ds(c, QB)] = _mm(dm_v[5 + r], y)
        return carry

    def inv9(t):
        ls = ds(t, 128)
        b0 = b9_v[0, 0:64, ls]
        br = [None] + [b9_v[r, 0:64, ls] for r in range(1, 5)]
        bi = [None] + [b9_v[r, 64:128, ls] for r in range(1, 5)]
        y = [None] * N1
        y[0] = b0 + br[1] + br[2] + br[3] + br[4]
        for d1 in range(1, 5):
            cc, ss = b0, None
            for r in range(1, 5):
                jr = (d1 * r) % N1
                co = _C9[min(jr, N1 - jr)]
                si = _S9[jr] if jr < 5 else -_S9[N1 - jr]
                cc = cc + br[r] * co
                ss = bi[r] * si if ss is None else ss + bi[r] * si
            y[d1] = cc - ss
            y[N1 - d1] = cc + ss
        yb = jnp.concatenate(y, axis=0).astype(BF16)
        for j in range(4):
            outa_v[ls, j * 128:(j + 1) * 128] = yb[j * 128:(j + 1) * 128].T
        tail_v[:, ls] = yb[512:576]

    def out_copy(c):
        return pltpu.make_async_copy(outb_v.at[ds(c, OB), :], out_hbm.at[ds(c, OB), pl.ds(512, 640)],
                                     osems.at[c])

    def outa_copy(t):
        return pltpu.make_async_copy(outa_v.at[ds(t, 128), :], out_hbm.at[ds(t, 128), pl.ds(0, 512)],
                                     osems.at[S // OB + t])

    cp_w.start()
    cp_xb(0).start()
    cp_xa(0).start()
    kt_v[D:D + 64, :] = jnp.zeros((64, S), BF16)
    for t in range(NT):
        z_v[t, 288:296, :] = jnp.zeros((8, 128), F32)
        z_v[t, RZ + 288:RZ + 296, :] = jnp.zeros((8, 128), F32)
    cp_w.wait()
    wt_v[0:D, :] = wqkv_v[:, D:2 * D].T
    wt_v[D:2 * D, :] = wqkv_v[:, 0:D].T
    late = [(cp_dm, cp_wv), (cp_wr, cp_wo), (cp_wi,), (cp_g,)]

    def p1(c, carry):
        cp_xb(c).wait()
        cp_xa(c).wait()

        @pl.when(c < NC - 1)
        def _():
            cp_xb(c + 1).start()
            cp_xa(c + 1).start()

        for cc, grp in enumerate(late):
            @pl.when(c == cc)
            def _():
                for cp in grp:
                    cp.start()
        _interleave(qk_units(c), fwd9_units(c))
        return carry
    lax.fori_loop(0, NC, p1, 0)
    for cp in (cp_dm, cp_wv, cp_wr, cp_wo, cp_wi):
        cp.wait()
    lax.fori_loop(0, NC, fwd64, 0)
    wt_v[2 * D:3 * D, :] = wqkv_v[:, 2 * D:3 * D].T
    wot_v[...] = wo_v[...].T
    fft16_v(0, -1)
    cp_g.wait()
    lax.fori_loop(0, NT // GU, gstep, 0)
    fft16_v(1, +1)
    lax.fori_loop(0, NC, inv64, 0)

    NK = S // KC
    PD = 2
    row_word = lax.broadcasted_iota(jnp.int32, (64, QB), 0)
    vrow = lax.broadcasted_iota(jnp.int32, (VR, KC), 0)

    def attn(i, carry):
        qb = i // NG
        g = i % NG
        q0 = pl.multiple_of(qb * QB, QB)
        r0 = pl.multiple_of(g * (HG * DH), 16)
        items = [(j, kc) for j in range(HG) for kc in range(NK)]
        qs, kws = {}, {}
        ps, accs, ms = {}, {}, {}
        outs = []

        def qk(it):
            j, kc = it
            if kc == 0:
                f = (g * HG + j) * DH
                w = f // 64
                f0 = pl.multiple_of(w * 64, 64)
                off = (f - f0) // 2
                qw = pltpu.bitcast(qt_v[pl.ds(f0, 128), pl.ds(q0, QB)], jnp.uint32)
                keep = (row_word >= off) & (row_word < off + DH // 2)
                qs[j] = pltpu.bitcast(jnp.where(keep, qw, jnp.uint32(0)), BF16)
                kws[j] = w
            s = _mm(kw_v[kws[j], kc * KC:(kc + 1) * KC, :], qs[j])
            mj = jnp.max(s, axis=0, keepdims=True)
            if kc == 0:
                alpha, mn = None, mj
            else:
                mn = jnp.maximum(ms[j], mj)
                alpha = jnp.exp2(ms[j] - mn)
            ms[j] = mn
            ps[it] = (jnp.exp2(s - mn).astype(BF16), alpha)

        def pv(it):
            j, kc = it
            p, alpha = ps.pop(it)
            lo = (j * DH) // 8 * 8
            hi = -((-(j + 1) * DH) // 8) * 8
            vs = vt_v[pl.ds(r0 + lo, hi - lo), kc * KC:(kc + 1) * KC]
            v24 = jnp.concatenate([vs[j * DH - lo:(j + 1) * DH - lo], jnp.zeros((VR - DH, KC), F32)], axis=0)
            v24 = jnp.where(vrow == DH, 1.0, v24)
            r = _mm(v24, p)
            accs[j] = r if kc == 0 else accs[j] * alpha + r
            if kc == NK - 1:
                a = accs.pop(j)
                outs.append(a[0:DH] * (1.0 / a[DH:DH + 1]))
                if j % 8 == 7:
                    ot_v[pl.ds(r0 + (j - 7) * DH, 8 * DH), pl.ds(q0, QB)] = (
                        jnp.concatenate(outs, axis=0).astype(BF16))
                    outs.clear()

        for n in range(PD):
            qk(items[n])
        for n in range(len(items)):
            if n + PD < len(items):
                qk(items[n + PD])
            pv(items[n])
            if n == 8:
                inv9(i)
        outa_copy(i).start()

        @pl.when(g == NG - 1)
        def _():
            def chunk(c, carry2):
                o = qb * (QB // OB) + c
                bt = _mm(wot_v[...], ot_v[:, ds(o, OB)]).astype(BF16)
                outb_v[ds(o, OB), 0:128] = jnp.concatenate([tail_v[:, ds(o, OB)], bt[0:64]], axis=0).T
                for j in range(1, 5):
                    outb_v[ds(o, OB), j * 128:(j + 1) * 128] = bt[j * 128 - 64:j * 128 + 64].T
                out_copy(o).start()
                return carry2
            lax.fori_loop(0, QB // OB, chunk, 0)
        return carry
    assert NG * NC == NT
    lax.fori_loop(0, NG * NC, attn, 0)
    for t in range(NT):
        outa_copy(t).wait()
    for c in range(S // OB):
        out_copy(c).wait()


@jax.jit
def pallas_concat_heads__spectral_gfnet__mha_block__prompt_kernel(
    A_x: jax.Array,
    A_w_r: jax.Array,
    A_w_i: jax.Array,
    B_x: jax.Array,
    B_wqkv: jax.Array,
    B_wo: jax.Array,
):
    dm, g = _constants()
    hbm = pl.BlockSpec(memory_space=pltpu.HBM)
    out = pl.pallas_call(
        _kernel,
        in_specs=[hbm] * 8,
        out_specs=hbm,
        out_shape=jax.ShapeDtypeStruct((S, 2 * D), BF16),
        scratch_shapes=[
            pltpu.VMEM((D, S), BF16),
            pltpu.VMEM((DF, S), BF16),
            pltpu.VMEM((DF, S), BF16),
            pltpu.VMEM((D, S), BF16),
            pltpu.VMEM((D, 3 * D), BF16),
            pltpu.VMEM((D, D), BF16),
            pltpu.VMEM((10, 128, 128), BF16),
            pltpu.VMEM((NT, 2, 128, 128), BF16),
            pltpu.VMEM((3 * D, D), BF16),
            pltpu.VMEM((D, D), BF16),
            pltpu.VMEM((640, S), BF16),
            pltpu.VMEM((640, S), BF16),
            pltpu.VMEM((9, S, 128), BF16),
            pltpu.VMEM((D, S), F32),
            pltpu.VMEM((D, S), BF16),
            pltpu.VMEM((5, 128, S), BF16),
            pltpu.VMEM((5, 128, S), F32),
            pltpu.VMEM((NT, 2 * RZ, 128), F32),
            pltpu.VMEM((4, S, 128), jnp.uint32),
            pltpu.VMEM((64, S), BF16),
            pltpu.VMEM((S, 512), BF16),
            pltpu.VMEM((S, 640), BF16),
            pltpu.SemaphoreType.DMA((15,)),
            pltpu.SemaphoreType.DMA((S // OB + NT,)),
        ],
        compiler_params=pltpu.CompilerParams(vmem_limit_bytes=110 * 1024 * 1024),
        name="gfnet_mha",
    )(A_x.reshape(S, D).T, A_w_r.T, A_w_i.T, B_x.reshape(S, D).T, B_wqkv, B_wo,
      jnp.asarray(dm, BF16), jnp.asarray(g, BF16))
    return out.reshape(1, S, 2 * D)
```
